```python
import os as _os
_os.environ.setdefault("JAX_PLATFORMS", "cpu")
import jax
import jax.numpy as jnp

def _softmax(x, axis=-1):
    return jax.nn.softmax(x, axis=axis)
def _gelu(x):
    return jax.nn.gelu(x, approximate=True)
def _silu(x):
    return jax.nn.silu(x)
def _sigmoid(x):
    return jax.nn.sigmoid(x)
def _layernorm(x, axis=-1, eps=1e-5):
    m = jnp.mean(x, axis=axis, keepdims=True)
    v = jnp.var(x, axis=axis, keepdims=True)
    return (x - m) / jnp.sqrt(v + eps)
def _scatter_add(tgt, idx, src, axis=0):
    return tgt.at[idx].add(src)
def _segment_sum(src, seg, n):
    return jax.ops.segment_sum(src, seg, n)
class _Rng:
    def __init__(self, key):
        self._k = key
    def _next(self):
        self._k, sub = jax.random.split(self._k)
        return sub
    def normal(self, shape):
        return jax.random.normal(self._next(), shape, dtype=jnp.bfloat16)
    def randint(self, lo, hi, shape):
        return jax.random.randint(self._next(), shape, lo, hi, dtype=jnp.int32)
    def uniform(self, shape, lo=0.0, hi=1.0):
        return jax.random.uniform(self._next(), shape, jnp.bfloat16, lo, hi)
    def permutation(self, n):
        return jax.random.permutation(self._next(), n)


kernel_name = 'interleave_layers__linear_attn_block__mha_block__prompt'

def setup_inputs():
    _rng = _Rng(jax.random.key(int.from_bytes(__import__("os").urandom(4), "little")))
    _w = (lambda a: (lambda t: t.astype(jnp.bfloat16) if jnp.issubdtype(t.dtype, jnp.floating) else t)(jnp.asarray(a)))
    def _A_setup():
        B, S, D = 1, 2048, 1024
        return {
            "x": _w((lambda *s: _rng.normal(s) * 0.05)(B, S, D)),
            "wqkv": _w((lambda *s: _rng.normal(s) * 0.1)(D, 3 * D)),
            "wo": _w((lambda *s: _rng.normal(s) * 0.1)(D, D)),
        }
    _A_in = _A_setup()

    def _B_setup():
        B, S, D, H = 1, 2048, 1024, 32
        return {
            "x": _w((lambda *s: _rng.normal(s) * 0.05)(B, S, D)),
            "wqkv": _w((lambda *s: _rng.normal(s) * 0.1)(D, 3 * D)),
            "wo": _w((lambda *s: _rng.normal(s) * 0.05)(D, D)),
        }
    _B_in = _B_setup()

    return {
        "A_x": _A_in["x"],
        "A_wqkv": _A_in["wqkv"],
        "A_wo": _A_in["wo"],
        "B_x": _B_in["x"],
        "B_wqkv": _B_in["wqkv"],
        "B_wo": _B_in["wo"],
    }

def reference(A_x, A_wqkv, A_wo, B_x, B_wqkv, B_wo):
    def _A_ref(x, wqkv, wo):
        B, S, D = x.shape
        H = 32; Dh = D // H
        qkv = (lambda x, *d: x.transpose(*d))((x @ wqkv).reshape(B, S, 3, H, Dh), 2, 0, 3, 1, 4)
        q, k, v = qkv[0], qkv[1], qkv[2]
        phi = lambda t: jnp.where(t > 0, t + 1, jnp.exp(t)) + 1e-6
        pq, pk = phi(q), phi(k)
        kv = jnp.einsum("bhsd,bhse->bhde", pk, v)
        z = jnp.einsum("bhsd->bhd", pk)
        num = jnp.einsum("bhqd,bhde->bhqe", pq, kv)
        den = jnp.einsum("bhqd,bhd->bhq", pq, z)[..., None] + 1e-6
        o = num / den
        return (lambda x, *d: x.transpose(*d))(o, 0, 2, 1, 3).reshape(B, S, D) @ wo

    def _B_ref(x, wqkv, wo):
        B, S, D = x.shape
        H = 32
        Dh = D // H
        qkv = (lambda x, *d: x.transpose(*d))((x @ wqkv).reshape(B, S, 3, H, Dh), 2, 0, 3, 1, 4)
        q, k, v = qkv[0], qkv[1], qkv[2]
        scores = jnp.einsum("bhqd,bhkd->bhqk", q, k) * (Dh ** -0.5)
        p = _softmax(scores, axis=-1)
        o = jnp.einsum("bhqk,bhkd->bhqd", p, v)
        return (lambda x, *d: x.transpose(*d))(o, 0, 2, 1, 3).reshape(B, S, D) @ wo

    x = A_x
    x = x + _A_ref(_layernorm(x, axis=-1), A_wqkv, A_wo)
    x = x + _B_ref(_layernorm(x, axis=-1), B_wqkv, B_wo)
    x = x + _A_ref(_layernorm(x, axis=-1), A_wqkv, A_wo)
    x = x + _B_ref(_layernorm(x, axis=-1), B_wqkv, B_wo)
    return x
```

```python
import contextlib
import math

import jax
import jax.numpy as jnp
from jax import lax
import jax.experimental.pallas as pl
import jax.experimental.pallas.tpu as pltpu

S, D, H, DH = 2048, 1024, 32, 32
NG = D // 128
TS = 512
SUB = 256
NSUB = TS // SUB
NT = S // TS
NX = S // SUB
TQ = 512
TK = 128
NQ = S // TQ
NC = S // TK
NIT = NG * NQ
WCHUNKS = ((0, 512), (512, 512), (1024, 1024), (2048, 1024))
QSCALE = (DH ** -0.5) * math.log2(math.e)
F32 = jnp.float32
BF16 = jnp.bfloat16
SCOPES = False


def _scope(name):
    return jax.named_scope(name) if SCOPES else contextlib.nullcontext()


def _dot(a, b):
    return jnp.dot(a, b, preferred_element_type=F32)


def _layernorm(x):
    mu = jnp.mean(x, axis=-1, keepdims=True)
    xc = x - mu
    var = jnp.mean(xc * xc, axis=-1, keepdims=True)
    return (xc * lax.rsqrt(var + 1e-5)).astype(BF16)


def _phi(t):
    return jnp.where(t > 0, t + 1.0, jnp.exp(t)) + 1e-6


def _recip(d):
    r = pl.reciprocal(d, approx=True)
    return r * (2.0 - d * r)


def _mult(v, m):
    return v if isinstance(v, int) else pl.multiple_of(v, m)


def _kernel(x_hbm, awqkv_hbm, awo_hbm, bwqkv_hbm, bwo_hbm, out_hbm,
            xio, awqkv, awo, bwqkv, bwo,
            x_s, pq_s, k_s, qt_s, vt_s, o_s, ott,
            kv_s, z_s, kvz_s,
            s0, s1, s2, s3, m_s, sems, wsems, xsems, osems):
    sb = (s0, s1, s2, s3)

    def x_copy(i):
        t0 = _mult(i * SUB, SUB)
        return pltpu.make_async_copy(x_hbm.at[pl.ds(t0, SUB)], xio.at[pl.ds(t0, SUB)], xsems.at[i])

    def w_copy(n):
        c0, w = WCHUNKS[n]
        return pltpu.make_async_copy(awqkv_hbm.at[:, pl.ds(c0, w)],
                                     awqkv.at[:, pl.ds(c0, w)], wsems.at[n])

    cp_awo = pltpu.make_async_copy(awo_hbm, awo, sems.at[0])
    cp_bwqkv = pltpu.make_async_copy(bwqkv_hbm, bwqkv, sems.at[1])
    cp_bwo = pltpu.make_async_copy(bwo_hbm, bwo, sems.at[2])
    x_copy(0).start()
    w_copy(0).start()

    def a_q(h, r0, c0=0, w=D):
        q = _dot(h, awqkv[:, c0:c0 + w])
        pq_s[pl.ds(r0, SUB), c0:c0 + w] = _phi(q).astype(BF16)

    def a_k(h):
        pk = _phi(_dot(h, awqkv[:, D:2 * D]))
        z_s[...] += jnp.sum(pk.reshape(SUB // 8, 8, D), axis=0)
        return pk.T.astype(BF16)

    def a_v(h, pkt):
        v = _dot(h, awqkv[:, 2 * D:3 * D]).astype(BF16)
        for g in range(NG):
            sl = slice(g * 128, (g + 1) * 128)
            kv_s[g] += _dot(pkt[sl, :], v[:, sl])

    def qkv_a(hs):
        for h, r0 in hs:
            pkt = a_k(h)
            a_v(h, pkt)
            a_q(h, r0)

    def qkv_b(hs):
        for h, r0 in hs:
            v = _dot(h, bwqkv[:, 2 * D:3 * D])
            vt_s[:, pl.ds(r0, SUB)] = v.T.astype(BF16)
            q = _dot(h, bwqkv[:, 0:D]) * QSCALE
            qt_s[:, pl.ds(r0, SUB)] = q.T.astype(BF16)
            k_s[pl.ds(r0, SUB), :] = _dot(h, bwqkv[:, D:2 * D]).astype(BF16)

    def lin_o(r0):
        pq = pq_s[pl.ds(r0, SUB), :]
        outs = []
        for g in range(NG):
            nd = _dot(pq[:, g * 128:(g + 1) * 128], kvz_s[g])
            outs.append((nd[:, :128] * _recip(nd[:, 128:] + 1e-6)).astype(BF16))
        return jnp.concatenate(outs, axis=1)

    def zero_kv():
        kv_s[...] = jnp.zeros(kv_s.shape, F32)
        z_s[...] = jnp.zeros(z_s.shape, F32)

    def finish_kv():
        ri = lax.broadcasted_iota(jnp.int32, (128, 128), 0) // DH
        ci = lax.broadcasted_iota(jnp.int32, (128, 128), 1) // DH
        diag = ri == ci
        z = jnp.sum(z_s[...], axis=0, keepdims=True)
        for g in range(NG):
            zg = jnp.broadcast_to(z[:, g * 128:(g + 1) * 128], (128, 128)).T
            kvz_s[g, :, 0:128] = jnp.where(diag, kv_s[g], 0.0).astype(BF16)
            kvz_s[g, :, 128:256] = jnp.where(diag, zg, 0.0).astype(BF16)

    def rows_of(i):
        t0 = _mult(i * TS, TS)
        return [_mult(t0 + u * SUB, SUB) for u in range(NSUB)]

    def ln_first(rs):
        for r0 in rs:
            x = xio[pl.ds(r0, SUB), :].astype(F32)
            x_s[pl.ds(r0, SUB), :] = x
            o_s[pl.ds(r0, SUB), :] = _layernorm(x)

    def pre_lin(rs):
        os_ = [lin_o(r0) for r0 in rs]
        hs = []
        for o, r0 in zip(os_, rs):
            x = x_s[pl.ds(r0, SUB), :] + _dot(o, awo[...])
            x_s[pl.ds(r0, SUB), :] = x
            hs.append((_layernorm(x), r0))
        return hs

    def pre_mha(rs):
        hs = []
        for r0 in rs:
            x = x_s[pl.ds(r0, SUB), :] + _dot(o_s[pl.ds(r0, SUB), :], bwo[...])
            x_s[pl.ds(r0, SUB), :] = x
            hs.append((_layernorm(x), r0))
        return hs

    def proj_phase(pre, post):
        def body(i, c):
            post(pre(rows_of(i)))
            return c
        lax.fori_loop(0, NT, body, 0)

    def make_w(g, j, q0):
        r0 = _mult(g * 128 + j * DH, DH)
        qh = qt_s[pl.ds(r0, DH), pl.ds(q0, TQ)]
        parts = []
        if j > 0:
            parts.append(jnp.zeros((DH * j, TQ), BF16))
        parts.append(qh)
        if j < 3:
            parts.append(jnp.zeros((DH * (3 - j), TQ), BF16))
        return jnp.concatenate(parts, axis=0)

    def s1_dot(c, w, l0):
        kc = k_s[pl.ds(c * TK, TK), pl.ds(l0, 128)]
        return _dot(kc, w)

    def s1_store(c, s, sbuf, m8):
        sbuf[pl.ds(c * TK, TK), :] = s
        for r in range(TK // 8):
            blk = s[r * 8:(r + 1) * 8, :]
            m8 = blk if m8 is None else jnp.maximum(m8, blk)
        return m8

    def s2_chunk(c, m, r0, sbuf, l8, acc):
        s = sbuf[pl.ds(c * TK, TK), :]
        p = jnp.exp2(s - m)
        for t in range(TK // 128):
            for r in reversed(range(8)):
                b0 = t * 128 + r * 16
                ab = p[b0:b0 + 8, :] + p[b0 + 8:b0 + 16, :]
                l8 = ab if l8 is None else l8 + ab
        vh = vt_s[pl.ds(r0, DH), pl.ds(c * TK, TK)]
        o = _dot(vh, p.astype(BF16))
        acc = o if acc is None else acc + o
        return l8, acc

    def item(it):
        g = it // NQ
        return g, _mult((it % NQ) * TQ, TQ)

    def flush_o(prev):
        g, q0 = prev
        o_s[pl.ds(q0, TQ), pl.ds(_mult(g * 128, 128), 128)] = ott[...].T.astype(BF16)

    def attn_step(prev, cur, nxt):
        if prev is not None:
            flush_o(prev)
        if cur is not None:
            g, q0 = cur
        if nxt is not None:
            gn, qn0 = nxt
            l0 = _mult(gn * 128, 128)
        for j in range(4):
            if cur is not None:
                r0 = _mult(g * 128 + j * DH, DH)
                m = m_s[j, 0:1, :]
            if nxt is not None:
                w = make_w(gn, j, qn0)
            m8 = None
            l8 = None
            acc = None
            for c in range(NC):
                if nxt is not None:
                    s = s1_dot(c, w, l0)
                if cur is not None:
                    l8, acc = s2_chunk(c, m, r0, sb[j], l8, acc)
                if nxt is not None:
                    m8 = s1_store(c, s, sb[j], m8)
            if cur is not None:
                l = jnp.sum(l8, axis=0, keepdims=True)
                ott[j * DH:(j + 1) * DH, :] = acc * _recip(l)
            if nxt is not None:
                m_s[j] = jnp.broadcast_to(jnp.max(m8, axis=0, keepdims=True), (8, TQ))

    def attention(first=False):
        with _scope("mha_pro"):
            attn_step(None, None, item(0))
            ott[...] = jnp.zeros(ott.shape, F32)

        def body(it, c):
            if first:
                @pl.when(it == 2)
                def _():
                    cp_bwo.start()
            attn_step(item(jnp.maximum(it - 1, 0)), item(it), item(it + 1))
            return c
        lax.fori_loop(0, NIT - 1, body, 0)
        with _scope("mha_epi"):
            attn_step(item(NIT - 2), item(NIT - 1), None)
            flush_o(item(NIT - 1))

    with _scope("P0a"):
        zero_kv()
        x_copy(0).wait()
        w_copy(1).start()
        ln_first([0])
        h = o_s[0:SUB, :]
        w_copy(0).wait()
        w_copy(2).start()
        a_q(h, 0, *WCHUNKS[0])
        w_copy(1).wait()
        w_copy(3).start()
        a_q(h, 0, *WCHUNKS[1])
        w_copy(2).wait()
        x_copy(1).start()
        pkt = a_k(h)
        w_copy(3).wait()
        x_copy(1).wait()
        for i in range(2, NX):
            x_copy(i).start()
        ln_first([SUB])
        a_v(h, pkt)

    def p0_body(i, c):
        inext = jnp.minimum(i + 1, NX - 1)

        @pl.when(i + 1 < NX)
        def _():
            x_copy(inext).wait()

        @pl.when(i == 2)
        def _():
            cp_awo.start()
            cp_bwqkv.start()
        r0 = _mult(i * SUB, SUB)
        qkv_a([(o_s[pl.ds(r0, SUB), :], r0)])
        ln_first([_mult(inext * SUB, SUB)])
        return c
    with _scope("P0"):
        lax.fori_loop(1, NX, p0_body, 0)
    cp_awo.wait()
    cp_bwqkv.wait()
    finish_kv()
    with _scope("P1"):
        proj_phase(pre_lin, qkv_b)
    with _scope("MHA"):
        attention(first=True)
    zero_kv()
    cp_bwo.wait()
    with _scope("P2"):
        proj_phase(pre_mha, qkv_a)
    finish_kv()
    with _scope("P1"):
        proj_phase(pre_lin, qkv_b)
    with _scope("MHA"):
        attention()

    def out_copy(i):
        t0 = _mult(i * TS, TS)
        return pltpu.make_async_copy(xio.at[pl.ds(t0, TS)], out_hbm.at[pl.ds(t0, TS)], osems.at[i])

    def final_body(i, c):
        for r0 in rows_of(i):
            y = x_s[pl.ds(r0, SUB), :] + _dot(o_s[pl.ds(r0, SUB), :], bwo[...])
            xio[pl.ds(r0, SUB), :] = y.astype(BF16)
        out_copy(i).start()
        return c
    with _scope("P4"):
        lax.fori_loop(0, NT, final_body, 0)

    with _scope("waitout"):
        for i in range(NT):
            out_copy(i).wait()


@jax.jit
def pallas_interleave_layers__linear_attn_block__mha_block__prompt_kernel(
    A_x: jax.Array,
    A_wqkv: jax.Array,
    A_wo: jax.Array,
    B_x: jax.Array,
    B_wqkv: jax.Array,
    B_wo: jax.Array,
):
    del B_x
    x = A_x.reshape(S, D)
    any_spec = pl.BlockSpec(memory_space=pl.ANY)
    out = pl.pallas_call(
        _kernel,
        out_shape=jax.ShapeDtypeStruct((S, D), BF16),
        in_specs=[any_spec] * 5,
        out_specs=any_spec,
        scratch_shapes=[
            pltpu.VMEM((S, D), BF16),
            pltpu.VMEM((D, 3 * D), BF16),
            pltpu.VMEM((D, D), BF16),
            pltpu.VMEM((D, 3 * D), BF16),
            pltpu.VMEM((D, D), BF16),
            pltpu.VMEM((S, D), F32),
            pltpu.VMEM((S, D), BF16),
            pltpu.VMEM((S, D), BF16),
            pltpu.VMEM((D, S), BF16),
            pltpu.VMEM((D, S), BF16),
            pltpu.VMEM((S, D), BF16),
            pltpu.VMEM((128, TQ), F32),
            pltpu.VMEM((NG, 128, 128), F32),
            pltpu.VMEM((8, D), F32),
            pltpu.VMEM((NG, 128, 256), BF16),
            pltpu.VMEM((S, TQ), F32),
            pltpu.VMEM((S, TQ), F32),
            pltpu.VMEM((S, TQ), F32),
            pltpu.VMEM((S, TQ), F32),
            pltpu.VMEM((4, 8, TQ), F32),
            pltpu.SemaphoreType.DMA((3,)),
            pltpu.SemaphoreType.DMA((len(WCHUNKS),)),
            pltpu.SemaphoreType.DMA((NX,)),
            pltpu.SemaphoreType.DMA((NT,)),
        ],
        compiler_params=pltpu.CompilerParams(vmem_limit_bytes=110 * 1024 * 1024),
        name="interleave_layers",
    )(x, A_wqkv, A_wo, B_wqkv, B_wo)
    return out.reshape(1, S, D)
```

```python
import contextlib
import math

import jax
import jax.numpy as jnp
from jax import lax
import jax.experimental.pallas as pl
import jax.experimental.pallas.tpu as pltpu

S, D, H, DH = 2048, 1024, 32, 32
NG = D // 128
TS = 512
SUB = 256
NSUB = TS // SUB
NT = S // TS
NX = S // SUB
CW = 256
NCW = D // CW
LNR = 32
TQ = 512
TK = 128
NQ = S // TQ
NC = S // TK
NIT = NG * NQ
WCHUNKS = ((1024, 256), (1280, 256), (1536, 512), (2048, 512), (2560, 512), (0, 512), (512, 512))
QSCALE = (DH ** -0.5) * math.log2(math.e)
F32 = jnp.float32
BF16 = jnp.bfloat16
SCOPES = False


def _scope(name):
    return jax.named_scope(name) if SCOPES else contextlib.nullcontext()


def _dot(a, b):
    return jnp.dot(a, b, preferred_element_type=F32)


def _layernorm(x):
    mu = jnp.mean(x, axis=-1, keepdims=True)
    xc = x - mu
    var = jnp.mean(xc * xc, axis=-1, keepdims=True)
    return (xc * lax.rsqrt(var + 1e-5)).astype(BF16)


def _ln_finish(x, s1, s2):
    mu = jnp.sum(s1, axis=-1, keepdims=True) * (1.0 / D)
    ms = jnp.sum(s2, axis=-1, keepdims=True) * (1.0 / D)
    var = jnp.maximum(ms - mu * mu, 0.0)
    return ((x - mu) * lax.rsqrt(var + 1e-5)).astype(BF16)


def _phi(t):
    return jnp.where(t > 0, t + 1.0, jnp.exp(t)) + 1e-6


def _recip(d):
    r = pl.reciprocal(d, approx=True)
    return r * (2.0 - d * r)


def _mult(v, m):
    return v if isinstance(v, int) else pl.multiple_of(v, m)


def _interleave(main, side):
    done = 0
    for n, task in enumerate(main):
        task()
        want = ((n + 1) * len(side)) // len(main)
        while done < want:
            side[done]()
            done += 1


def _kernel(x_hbm, awqkv_hbm, awo_hbm, bwqkv_hbm, bwo_hbm, out_hbm,
            xio, awqkv, awo, bwqkv, bwo,
            x_s, pq_s, k_s, qt_s, vt_s, o_s, ott,
            kv_s, z_s, zc_s, kvw_s, pqt_s,
            s0, s1, s2, s3, m_s, sems, wsems, xsems, osems):
    sb = (s0, s1, s2, s3)

    def x_copy(i):
        t0 = _mult(i * SUB, SUB)
        return pltpu.make_async_copy(x_hbm.at[pl.ds(t0, SUB)], xio.at[pl.ds(t0, SUB)], xsems.at[i])

    def w_copy(n):
        c0, w = WCHUNKS[n]
        return pltpu.make_async_copy(awqkv_hbm.at[:, pl.ds(c0, w)],
                                     awqkv.at[:, pl.ds(c0, w)], wsems.at[n])

    cp_awo = pltpu.make_async_copy(awo_hbm, awo, sems.at[0])
    cp_bwqkv = pltpu.make_async_copy(bwqkv_hbm, bwqkv, sems.at[1])
    cp_bwo = pltpu.make_async_copy(bwo_hbm, bwo, sems.at[2])
    x_copy(0).start()
    w_copy(0).start()

    def qkv_a_tasks(get_h, r0):
        st = {}

        def k_task(n):
            def f():
                c0 = n * CW
                pk = _phi(_dot(get_h(), awqkv[:, D + c0:D + c0 + CW]))
                z_s[:, c0:c0 + CW] += jnp.sum(pk.reshape(SUB // 8, 8, CW), axis=0)
                st["k", n] = pk.T.astype(BF16)
            return f

        def v_task(n):
            def f():
                c0 = n * CW
                st["v", n] = _dot(get_h(), awqkv[:, 2 * D + c0:2 * D + c0 + CW]).astype(BF16)
            return f

        def q_task(n):
            def f():
                c0 = n * CW
                q = _dot(get_h(), awqkv[:, c0:c0 + CW])
                pqt_s[c0:c0 + CW, pl.ds(r0, SUB)] = _phi(q).T.astype(BF16)
            return f

        def kv_task():
            for g in range(NG):
                n, o = divmod(g * 128, CW)
                kv_s[g] += _dot(st["k", n][o:o + 128, :], st["v", n][:, o:o + 128])

        return ([k_task(n) for n in range(NCW)] + [v_task(n) for n in range(NCW)]
                + [q_task(n) for n in range(NCW)] + [kv_task])

    def qkv_b_tasks(get_h, r0):
        def v_task(n):
            def f():
                c0 = n * CW
                v = _dot(get_h(), bwqkv[:, 2 * D + c0:2 * D + c0 + CW])
                vt_s[c0:c0 + CW, pl.ds(r0, SUB)] = v.T.astype(BF16)
            return f

        def q_task(n):
            def f():
                c0 = n * CW
                q = _dot(get_h(), bwqkv[:, c0:c0 + CW]) * QSCALE
                qt_s[c0:c0 + CW, pl.ds(r0, SUB)] = q.T.astype(BF16)
            return f

        def k_task(n):
            def f():
                c0 = n * CW
                k_s[pl.ds(r0, SUB), c0:c0 + CW] = _dot(
                    get_h(), bwqkv[:, D + c0:D + c0 + CW]).astype(BF16)
            return f

        return ([v_task(n) for n in range(NCW)] + [q_task(n) for n in range(NCW)]
                + [k_task(n) for n in range(NCW)])

    def out_tasks(lhs_ref, w_ref, r0):
        xs, st = [], {}

        def mm(n):
            def f():
                c0 = n * CW
                x = x_s[pl.ds(r0, SUB), c0:c0 + CW] + _dot(
                    lhs_ref[pl.ds(r0, SUB), :], w_ref[:, c0:c0 + CW])
                x_s[pl.ds(r0, SUB), c0:c0 + CW] = x
                xs.append(x)
                for u in range(CW // 128):
                    xu = x[:, u * 128:(u + 1) * 128]
                    st["s1"] = xu if "s1" not in st else st["s1"] + xu
                    st["s2"] = xu * xu if "s2" not in st else st["s2"] + xu * xu
            return f

        def get_h():
            if "h" not in st:
                st["h"] = _ln_finish(jnp.concatenate(xs, axis=1), st["s1"], st["s2"])
            return st["h"]

        return [mm(n) for n in range(NCW)], get_h

    def norm_pq_tasks(t0):
        def task(u, n):
            def f():
                c0 = _mult(t0 + u * 128, 128)
                nh = CW // DH
                rows = slice(n * CW, (n + 1) * CW)
                pqt = pqt_s[rows, pl.ds(c0, 128)].astype(F32).reshape(nh, DH, 128)
                den = jnp.sum(pqt * zc_s[rows, :].reshape(nh, DH, 128), axis=1, keepdims=True) + 1e-6
                pn = (pqt * _recip(den)).reshape(CW, 128)
                pq_s[pl.ds(c0, 128), rows] = pn.T.astype(BF16)
            return f
        return [task(u, n) for u in range(TS // 128) for n in range(NCW)]

    def zero_kv():
        kv_s[...] = jnp.zeros(kv_s.shape, F32)
        z_s[...] = jnp.zeros(z_s.shape, F32)

    def finish_kv():
        ri = lax.broadcasted_iota(jnp.int32, (128, 128), 0) // DH
        ci = lax.broadcasted_iota(jnp.int32, (128, 128), 1) // DH
        diag = ri == ci
        z = jnp.sum(z_s[...], axis=0, keepdims=True)
        zc_s[...] = jnp.broadcast_to(z, (128, D)).T

        def kvw(g):
            def f():
                sl = slice(g * 128, (g + 1) * 128)
                kvd = jnp.where(diag, kv_s[g], 0.0).astype(BF16)
                kvw_s[sl, :] = _dot(kvd, awo[sl, :]).astype(BF16)
            return f
        _interleave([kvw(g) for g in range(NG)], norm_pq_tasks(0))

    def rows_of(i):
        t0 = _mult(i * TS, TS)
        return [_mult(t0 + u * SUB, SUB) for u in range(NSUB)]

    def ln_first_tasks(r0):
        def task(p):
            def f():
                rr = _mult(r0 + p * LNR, LNR)
                x = xio[pl.ds(rr, LNR), :].astype(F32)
                x_s[pl.ds(rr, LNR), :] = x
                o_s[pl.ds(rr, LNR), :] = _layernorm(x)
            return f
        return [task(p) for p in range(SUB // LNR)]

    def proj_phase(lhs_ref, w_ref, qkv_tasks, lin):
        def body(i, c):
            ra, rb = rows_of(i)
            mm_a, h_a = out_tasks(lhs_ref, w_ref, ra)
            mm_b, h_b = out_tasks(lhs_ref, w_ref, rb)
            side = norm_pq_tasks(_mult(jnp.minimum(i + 1, NT - 1) * TS, TS)) if lin else []
            _interleave(mm_a, [])
            h_a()
            _interleave(mm_b, [])
            h_b()
            for t in side:
                t()
            _interleave(qkv_tasks(h_a, ra), [])
            _interleave(qkv_tasks(h_b, rb), [])
            return c
        lax.fori_loop(0, NT, body, 0)

    def make_w(g, j, q0):
        r0 = _mult(g * 128 + j * DH, DH)
        qh = qt_s[pl.ds(r0, DH), pl.ds(q0, TQ)]
        parts = []
        if j > 0:
            parts.append(jnp.zeros((DH * j, TQ), BF16))
        parts.append(qh)
        if j < 3:
            parts.append(jnp.zeros((DH * (3 - j), TQ), BF16))
        return jnp.concatenate(parts, axis=0)

    def s1_dot(c, w, l0):
        kc = k_s[pl.ds(c * TK, TK), pl.ds(l0, 128)]
        return _dot(kc, w)

    def s1_store(c, s, sbuf, m8):
        sbuf[pl.ds(c * TK, TK), :] = s
        for r in range(TK // 8):
            blk = s[r * 8:(r + 1) * 8, :]
            m8 = blk if m8 is None else jnp.maximum(m8, blk)
        return m8

    def s2_chunk(c, m, r0, sbuf, l8, acc):
        s = sbuf[pl.ds(c * TK, TK), :]
        p = jnp.exp2(s - m)
        for t in range(TK // 128):
            for r in reversed(range(8)):
                b0 = t * 128 + r * 16
                ab = p[b0:b0 + 8, :] + p[b0 + 8:b0 + 16, :]
                l8 = ab if l8 is None else l8 + ab
        vh = vt_s[pl.ds(r0, DH), pl.ds(c * TK, TK)]
        o = _dot(vh, p.astype(BF16))
        acc = o if acc is None else o + acc
        return l8, acc

    def item(it):
        return it % NG, _mult((it // NG) * TQ, TQ)

    def flush_o(prev):
        g, q0 = prev
        o_s[pl.ds(q0, TQ), pl.ds(_mult(g * 128, 128), 128)] = ott[...].T.astype(BF16)

    def attn_step(prev, cur, nxt, extra=()):
        extra = list(extra)
        every = (4 * NC) // len(extra) if extra else 0
        if prev is not None:
            flush_o(prev)
        if cur is not None:
            g, q0 = cur
        if nxt is not None:
            gn, qn0 = nxt
            l0 = _mult(gn * 128, 128)
        for j in range(4):
            if cur is not None:
                r0 = _mult(g * 128 + j * DH, DH)
                m = m_s[j, 0:1, :]
            if nxt is not None:
                w = make_w(gn, j, qn0)
            m8 = None
            l8 = None
            acc = None
            for c in range(NC):
                if extra and (j * NC + c) % every == 0:
                    extra.pop(0)()
                if nxt is not None:
                    s = s1_dot(c, w, l0)
                if cur is not None:
                    l8, acc = s2_chunk(c, m, r0, sb[j], l8, acc)
                if nxt is not None:
                    m8 = s1_store(c, s, sb[j], m8)
            if cur is not None:
                l = jnp.sum(l8, axis=0, keepdims=True)
                ott[j * DH:(j + 1) * DH, :] = acc * _recip(l)
            if nxt is not None:
                m_s[j] = jnp.broadcast_to(jnp.max(m8, axis=0, keepdims=True), (8, TQ))

    def attention(first=False, extra=()):
        with _scope("mha_pro"):
            attn_step(None, None, item(0))
            ott[...] = jnp.zeros(ott.shape, F32)

        def body(it, c):
            if first:
                @pl.when(it == 2)
                def _():
                    cp_bwo.start()
            attn_step(item(jnp.maximum(it - 1, 0)), item(it), item(it + 1))
            return c
        lax.fori_loop(0, NIT - 1, body, 0)
        with _scope("mha_epi"):
            attn_step(item(NIT - 2), item(NIT - 1), None, extra)
            flush_o(item(NIT - 1))

    with _scope("P0a"):
        zero_kv()
        x_copy(0).wait()
        w_copy(1).start()
        for t in ln_first_tasks(0):
            t()
        h0 = o_s[0:SUB, :]
        tasks = qkv_a_tasks(lambda: h0, 0)
        nw = len(WCHUNKS)
        pos = 0
        for n in range(nw):
            w_copy(n).wait()
            if n + 2 < nw:
                w_copy(n + 2).start()
            if n == nw - 3:
                x_copy(1).start()
            side = []
            if n == nw - 1:
                x_copy(1).wait()
                for i in range(2, NX):
                    x_copy(i).start()
                side = ln_first_tasks(SUB)
            if n == nw - 2:
                tasks[-1]()
            per = WCHUNKS[n][1] // CW
            _interleave(tasks[pos:pos + per], side)
            pos += per

    def p0_body(i, c):
        inext = jnp.minimum(i + 1, NX - 1)

        @pl.when(i + 1 < NX)
        def _():
            x_copy(inext).wait()

        @pl.when(i == 2)
        def _():
            cp_awo.start()
            cp_bwqkv.start()
        r0 = _mult(i * SUB, SUB)
        h = o_s[pl.ds(r0, SUB), :]
        tasks = qkv_a_tasks(lambda: h, r0)
        _interleave(tasks[:-1], ln_first_tasks(_mult(inext * SUB, SUB)))
        tasks[-1]()
        return c
    with _scope("P0"):
        lax.fori_loop(1, NX, p0_body, 0)
    cp_awo.wait()
    cp_bwqkv.wait()
    finish_kv()
    with _scope("P1"):
        proj_phase(pq_s, kvw_s, qkv_b_tasks, True)
    with _scope("MHA"):
        attention(first=True)
    zero_kv()
    cp_bwo.wait()
    with _scope("P2"):
        proj_phase(o_s, bwo, qkv_a_tasks, False)
    finish_kv()
    with _scope("P1"):
        proj_phase(pq_s, kvw_s, qkv_b_tasks, True)

    def fin_pieces(r0, c0):
        st = {}

        def f0():
            st["p"] = _dot(o_s[r0:r0 + 128, 0:512], bwo[0:512, c0:c0 + 128]) + x_s[r0:r0 + 128, c0:c0 + 128]

        def f1():
            y = _dot(o_s[r0:r0 + 128, 512:1024], bwo[512:1024, c0:c0 + 128]) + st["p"]
            xio[r0:r0 + 128, c0:c0 + 128] = y.astype(BF16)
        return [f0, f1]

    with _scope("MHA"):
        attention(extra=[f for r0 in range(0, TS, 128) for c0 in range(0, D, 128)
                         for f in fin_pieces(r0, c0)])

    def out_copy(i):
        t0 = _mult(i * SUB, SUB)
        return pltpu.make_async_copy(xio.at[pl.ds(t0, SUB)], out_hbm.at[pl.ds(t0, SUB)], osems.at[i])

    def final_body(i, c):
        for u, r0 in enumerate(rows_of(i)):
            y = x_s[pl.ds(r0, SUB), :] + _dot(o_s[pl.ds(r0, SUB), :], bwo[...])
            xio[pl.ds(r0, SUB), :] = y.astype(BF16)
            out_copy(i * NSUB + u).start()
        return c
    for u in range(NSUB):
        out_copy(u).start()
    with _scope("P4"):
        lax.fori_loop(1, NT, final_body, 0)

    with _scope("waitout"):
        for i in range(NX):
            out_copy(i).wait()


@jax.jit
def pallas_interleave_layers__linear_attn_block__mha_block__prompt_kernel(
    A_x: jax.Array,
    A_wqkv: jax.Array,
    A_wo: jax.Array,
    B_x: jax.Array,
    B_wqkv: jax.Array,
    B_wo: jax.Array,
):
    del B_x
    x = A_x.reshape(S, D)
    any_spec = pl.BlockSpec(memory_space=pl.ANY)
    out = pl.pallas_call(
        _kernel,
        out_shape=jax.ShapeDtypeStruct((S, D), BF16),
        in_specs=[any_spec] * 5,
        out_specs=any_spec,
        scratch_shapes=[
            pltpu.VMEM((S, D), BF16),
            pltpu.VMEM((D, 3 * D), BF16),
            pltpu.VMEM((D, D), BF16),
            pltpu.VMEM((D, 3 * D), BF16),
            pltpu.VMEM((D, D), BF16),
            pltpu.VMEM((S, D), F32),
            pltpu.VMEM((S, D), BF16),
            pltpu.VMEM((S, D), BF16),
            pltpu.VMEM((D, S), BF16),
            pltpu.VMEM((D, S), BF16),
            pltpu.VMEM((S, D), BF16),
            pltpu.VMEM((128, TQ), F32),
            pltpu.VMEM((NG, 128, 128), F32),
            pltpu.VMEM((8, D), F32),
            pltpu.VMEM((D, 128), F32),
            pltpu.VMEM((D, D), BF16),
            pltpu.VMEM((D, S), BF16),
            pltpu.VMEM((S, TQ), F32),
            pltpu.VMEM((S, TQ), F32),
            pltpu.VMEM((S, TQ), F32),
            pltpu.VMEM((S, TQ), F32),
            pltpu.VMEM((4, 8, TQ), F32),
            pltpu.SemaphoreType.DMA((3,)),
            pltpu.SemaphoreType.DMA((len(WCHUNKS),)),
            pltpu.SemaphoreType.DMA((NX,)),
            pltpu.SemaphoreType.DMA((NX,)),
        ],
        compiler_params=pltpu.CompilerParams(vmem_limit_bytes=110 * 1024 * 1024),
        name="interleave_layers",
    )(x, A_wqkv, A_wo, B_wqkv, B_wo)
    return out.reshape(1, S, D)
```

```python
import contextlib
import math

import jax
import jax.numpy as jnp
from jax import lax
import jax.experimental.pallas as pl
import jax.experimental.pallas.tpu as pltpu

S, D, H, DH = 2048, 1024, 32, 32
NG = D // 128
TS = 512
SUB = 256
NSUB = TS // SUB
NT = S // TS
NX = S // SUB
CW = 256
NCW = D // CW
LNR = 32
TQ = 512
TK = 128
NQ = S // TQ
NC = S // TK
NIT = NG * NQ
LAG = 2
WCHUNKS = ((1024, 256), (1280, 256), (1536, 512), (2048, 512), (2560, 512), (0, 512), (512, 512))
QSCALE = (DH ** -0.5) * math.log2(math.e)
F32 = jnp.float32
BF16 = jnp.bfloat16
SCOPES = False


def _scope(name):
    return jax.named_scope(name) if SCOPES else contextlib.nullcontext()


def _dot(a, b):
    return jnp.dot(a, b, preferred_element_type=F32)


def _ln_finish(x, s1, s2):
    mu = jnp.sum(s1, axis=-1, keepdims=True) * (1.0 / D)
    ms = jnp.sum(s2, axis=-1, keepdims=True) * (1.0 / D)
    var = jnp.maximum(ms - mu * mu, 0.0)
    return ((x - mu) * lax.rsqrt(var + 1e-5)).astype(BF16)


def _layernorm(x):
    return _ln_finish(x, x, x * x)


def _phi(t):
    return jnp.where(t > 0, t + 1.0, jnp.exp(t)) + 1e-6


def _recip(d):
    r = pl.reciprocal(d, approx=True)
    return r * (2.0 - d * r)


def _mult(v, m):
    return v if isinstance(v, int) else pl.multiple_of(v, m)


def _pack(v):
    return pltpu.bitcast(v, jnp.uint32)


def _unpack(v):
    return pltpu.bitcast(v, BF16)


def _half(r0, n):
    return pl.ds(_mult(r0 // 2, n // 2), n // 2)


def _interleave(main, side):
    done = 0
    for n, task in enumerate(main):
        task()
        want = ((n + 1) * len(side)) // len(main)
        while done < want:
            side[done]()
            done += 1


def _kernel(x_hbm, awqkv_hbm, awo_hbm, bwqkv_hbm, bwo_hbm, out_hbm,
            xio, awqkv, awo, bwqkv, bwo,
            x_s, pq_s, k_s, qt_s, vt_s, o_s, ott,
            kv_s, z_s, zc_s, kvw_s, pqt_s, bwo_p, hb_s,
            m_s, sems, wsems, xsems, osems, *sb):

    def x_copy(i):
        t0 = _mult(i * SUB, SUB)
        return pltpu.make_async_copy(x_hbm.at[pl.ds(t0, SUB)], xio.at[pl.ds(t0, SUB)], xsems.at[i])

    def w_copy(n):
        c0, w = WCHUNKS[n]
        return pltpu.make_async_copy(awqkv_hbm.at[:, pl.ds(c0, w)],
                                     awqkv.at[:, pl.ds(c0, w)], wsems.at[n])

    cp_awo = pltpu.make_async_copy(awo_hbm, awo, sems.at[0])
    cp_bwqkv = pltpu.make_async_copy(bwqkv_hbm, bwqkv, sems.at[1])
    cp_bwo = pltpu.make_async_copy(bwo_hbm, bwo, sems.at[2])
    x_copy(0).start()
    w_copy(0).start()

    def qkv_a_tasks(get_h, i, u, split=False):
        st = {}

        def mm(key, c0):
            def f():
                st[key] = _dot(get_h(), awqkv[:, c0:c0 + CW])
            return f

        def k_post(n):
            def f():
                c0 = n * CW
                pk = _phi(st["k", n])
                z_s[:, c0:c0 + CW] += jnp.sum(pk.reshape(SUB // 8, 8, CW), axis=0)
                st["k", n] = pk.T.astype(BF16)
            return f

        def v_post(n):
            def f():
                st["v", n] = st["v", n].astype(BF16)
            return f

        def q_post(n):
            def f():
                c0 = n * CW
                pqt_s[i * NSUB + u, c0:c0 + CW, :] = _phi(st["q", n]).T.astype(BF16)
            return f

        def kv_task():
            for g in range(NG):
                n, o = divmod(g * 128, CW)
                kv_s[g] += _dot(st["k", n][o:o + 128, :], st["v", n][:, o:o + 128])

        pairs = ([(mm(("k", n), D + n * CW), k_post(n)) for n in range(NCW)]
                 + [(mm(("v", n), 2 * D + n * CW), v_post(n)) for n in range(NCW)]
                 + [(mm(("q", n), n * CW), q_post(n)) for n in range(NCW)])
        if split:
            return pairs, kv_task

        def both(p):
            def f():
                p[0]()
                p[1]()
            return f
        return [both(p) for p in pairs] + [kv_task]

    def qkv_b_tasks(get_h, i, u):
        r0 = rows_of(i)[u]
        cols = slice(u * SUB, (u + 1) * SUB)

        def v_task(n):
            def f():
                c0 = n * CW
                v = _dot(get_h(), bwqkv[:, 2 * D + c0:2 * D + c0 + CW])
                vt_s[i, c0:c0 + CW, cols] = v.T.astype(BF16)
            return f

        def q_task(n):
            def f():
                c0 = n * CW
                q = _dot(get_h(), bwqkv[:, c0:c0 + CW]) * QSCALE
                qt_s[i, c0:c0 + CW, cols] = q.T.astype(BF16)
            return f

        def k_task(n):
            def f():
                c0 = n * CW
                k = _dot(get_h(), bwqkv[:, D + c0:D + c0 + CW]).astype(BF16)
                for t in range(CW // 128):
                    k_s[c0 // 128 + t, pl.ds(r0, SUB), :] = k[:, t * 128:(t + 1) * 128]
            return f

        return ([v_task(n) for n in range(NCW)] + [q_task(n) for n in range(NCW)]
                + [k_task(n) for n in range(NCW)])

    def out_tasks(lhs, w_ref, r0, res_ref):
        xs, st = [], {}

        def mm(n):
            def f():
                c0 = n * CW
                x = res_ref[pl.ds(r0, SUB), c0:c0 + CW].astype(F32) + _dot(
                    lhs(r0, SUB), _unpack(w_ref[:, c0:c0 + CW]))
                x_s[pl.ds(r0, SUB), c0:c0 + CW] = x
                xs.append(x)
                for u in range(CW // 128):
                    xu = x[:, u * 128:(u + 1) * 128]
                    st["s1"] = xu if "s1" not in st else st["s1"] + xu
                    st["s2"] = xu * xu if "s2" not in st else st["s2"] + xu * xu
            return f

        def get_h():
            if "h" not in st:
                st["h"] = _ln_finish(jnp.concatenate(xs, axis=1), st["s1"], st["s2"])
            return st["h"]

        return [mm(n) for n in range(NCW)], get_h

    def lhs_pq(r0, n):
        return _unpack(pq_s[_half(r0, n), :])

    def lhs_o(r0, n, g0=0, g1=NG):
        h0 = _mult(r0 // 2, n // 2)
        return pltpu.bitcast(
            jnp.concatenate([o_s[g, pl.ds(h0, n // 2), :] for g in range(g0, g1)], axis=1), BF16)

    def norm_pq_tasks(i):
        def task(u, n):
            def f():
                c0 = _mult(i * TS + u * 128, 128)
                ix, lo = divmod(u * 128, SUB)
                nh = CW // DH
                rows = slice(n * CW, (n + 1) * CW)
                pqt = pqt_s[i * NSUB + ix, rows, lo:lo + 128].astype(F32).reshape(nh, DH, 128)
                den = jnp.sum(pqt * zc_s[rows, :].reshape(nh, DH, 128), axis=1, keepdims=True) + 1e-6
                pn = (pqt * _recip(den)).reshape(CW, 128)
                pq_s[_half(c0, 128), rows] = _pack(pn.T.astype(BF16))
            return f
        return [task(u, n) for u in range(TS // 128) for n in range(NCW)]

    def zero_kv():
        kv_s[...] = jnp.zeros(kv_s.shape, F32)
        z_s[...] = jnp.zeros(z_s.shape, F32)

    def finish_kv():
        ri = lax.broadcasted_iota(jnp.int32, (128, 128), 0) // DH
        ci = lax.broadcasted_iota(jnp.int32, (128, 128), 1) // DH
        diag = ri == ci
        z = jnp.sum(z_s[...], axis=0, keepdims=True)
        zc_s[...] = jnp.broadcast_to(z, (128, D)).T

        def kvw(g):
            def f():
                sl = slice(g * 128, (g + 1) * 128)
                kvd = jnp.where(diag, kv_s[g], 0.0).astype(BF16)
                kvw_s[g * 64:(g + 1) * 64, :] = _pack(_dot(kvd, awo[sl, :]).astype(BF16))
            return f
        _interleave([kvw(g) for g in range(NG)], norm_pq_tasks(0))

    def rows_of(i):
        t0 = _mult(i * TS, TS)
        return [_mult(t0 + u * SUB, SUB) for u in range(NSUB)]

    def ln_first_tasks(r0, src=xio, rows=SUB, dst=pq_s):
        def task(p):
            def f():
                rr = _mult(r0 + p * LNR, LNR)
                x = src[pl.ds(rr, LNR), :].astype(F32)
                dst[_half(rr, LNR), :] = _pack(_layernorm(x))
            return f
        return [task(p) for p in range(rows // LNR)]

    def proj_phase(lhs, w_ref, qkv_tasks, lin, res_ref):
        def body(i, c):
            ra, rb = rows_of(i)
            mm_a, h_a = out_tasks(lhs, w_ref, ra, res_ref)
            mm_b, h_b = out_tasks(lhs, w_ref, rb, res_ref)
            side = norm_pq_tasks(jnp.minimum(i + 1, NT - 1)) if lin else []
            _interleave(mm_a, [])
            h_a()
            _interleave(mm_b, [])
            h_b()
            for t in side:
                t()
            _interleave(qkv_tasks(h_a, i, 0), [])
            if res_ref is xio:
                w0 = _mult(i * (D // NT), D // NT)
                bwo_p[_half(w0, D // NT), :] = _pack(bwo[pl.ds(w0, D // NT), :])
            _interleave(qkv_tasks(h_b, i, 1), [])
            return c
        lax.fori_loop(0, NT, body, 0)

    def make_w(g, j, qi):
        r0 = _mult(g * 128 + j * DH, DH)
        qh = qt_s[qi, pl.ds(r0, DH), :]
        parts = []
        if j > 0:
            parts.append(jnp.zeros((DH * j, TQ), BF16))
        parts.append(qh)
        if j < 3:
            parts.append(jnp.zeros((DH * (3 - j), TQ), BF16))
        return jnp.concatenate(parts, axis=0)

    def s1_dot(c, w, g):
        kc = k_s[g, c * TK:(c + 1) * TK, :]
        return _dot(kc, w)

    def s1_store(c, s, sbuf, m8):
        sbuf[pl.ds(c * TK, TK), :] = s
        for r in range(TK // 8):
            blk = s[r * 8:(r + 1) * 8, :]
            m8 = blk if m8 is None else jnp.maximum(m8, blk)
        return m8

    def s2_chunk(c, m, r0, sbuf, l8, acc):
        s = sbuf[pl.ds(c * TK, TK), :]
        p = jnp.exp2(s - m)
        for t in range(TK // 128):
            for r in reversed(range(8)):
                b0 = t * 128 + r * 16
                ab = p[b0:b0 + 8, :] + p[b0 + 8:b0 + 16, :]
                l8 = ab if l8 is None else l8 + ab
        ti, lo = divmod(c * TK, TS)
        vh = vt_s[ti, pl.ds(r0, DH), lo:lo + TK]
        o = _dot(vh, p.astype(BF16))
        acc = o if acc is None else o + acc
        return l8, acc

    def item(it):
        return it % NG, it // NG

    def flush_o(prev, slot):
        g, qi = prev
        o_s[g, pl.ds(_mult(qi * (TQ // 2), TQ // 2), TQ // 2), :] = pltpu.bitcast(
            ott[slot].T.astype(BF16), jnp.uint32)

    def attn_step(prev, cur, nxt, slot, extra=()):
        extra = list(extra)
        every = (4 * NC) // len(extra) if extra else 0
        if prev is not None:
            flush_o(prev, slot)
        if cur is not None:
            g, _ = cur
        if nxt is not None:
            gn, qn = nxt
        for j in range(4):
            b = slot * 4 + j
            if cur is not None:
                r0 = _mult(g * 128 + j * DH, DH)
                m = m_s[b, 0:1, :]
            if nxt is not None:
                w = make_w(gn, j, qn)
            m8 = None
            l8 = None
            acc = None
            for c in range(NC):
                if extra and (j * NC + c) % every == 0:
                    extra.pop(0)()
                if nxt is not None:
                    s = s1_dot(c, w, gn)
                if cur is not None:
                    l8, acc = s2_chunk(c, m, r0, sb[b], l8, acc)
                if nxt is not None:
                    m8 = s1_store(c, s, sb[b], m8)
            if cur is not None:
                l = jnp.sum(l8, axis=0, keepdims=True)
                ott[slot, j * DH:(j + 1) * DH, :] = acc * _recip(l)
            if nxt is not None:
                m_s[b] = jnp.broadcast_to(jnp.max(m8, axis=0, keepdims=True), (8, TQ))

    def attention(lag, first, extra):
        with _scope("mha_pro"):
            for u in range(lag):
                attn_step(None, None, item(u), u)
            ott[...] = jnp.zeros(ott.shape, F32)
            if first:
                zero_kv()

        def body(ib, c):
            for u in range(lag):
                it = ib * lag + u
                attn_step(item(jnp.maximum(ib - 1, 0) * lag + u), item(it), item(it + lag), u)
            return c
        lax.fori_loop(0, NIT // lag - 1, body, 0)
        with _scope("mha_epi"):
            ne = len(extra) // lag
            for u in range(lag):
                it = NIT - lag + u
                attn_step(item(it - lag), item(it), None, u, extra[u * ne:(u + 1) * ne])
            for u in range(lag):
                flush_o(item(NIT - lag + u), u)

    def fin_pieces(r0, c0, last, PR):
        st = {}

        def f0():
            st["p"] = (_dot(lhs_o(r0, PR, 0, 4), _unpack(bwo_p[0:256, c0:c0 + 128]))
                       + x_s[r0:r0 + PR, c0:c0 + 128])

        def f1():
            y = _dot(lhs_o(r0, PR, 4, 8), _unpack(bwo_p[256:512, c0:c0 + 128])) + st["p"]
            if last:
                xio[r0:r0 + PR, c0:c0 + 128] = y.astype(BF16)
            else:
                x_s[r0:r0 + PR, c0:c0 + 128] = y
                if c0 + 128 == D:
                    for t in ln_first_tasks(r0, x_s, PR, (pq_s, hb_s)[(r0 // SUB) % 2]):
                        t()
        return [f0, f1]

    def fin_extra(last, lag):
        pr = 128 // lag
        return [f for r0 in range(0, TS, pr) for c0 in range(0, D, 128)
                for f in fin_pieces(r0, c0, last, pr)]

    with _scope("P0a"):
        zero_kv()
        x_copy(0).wait()
        w_copy(1).start()
        for t in ln_first_tasks(0):
            t()
        h0 = lhs_pq(0, SUB)
        pairs, kv_task = qkv_a_tasks(lambda: h0, 0, 0, split=True)
        nw = len(WCHUNKS)
        pos = 0
        pending = []
        for n in range(nw):
            w_copy(n).wait()
            if n + 2 < nw:
                w_copy(n + 2).start()
            if n == nw - 3:
                x_copy(1).start()
            if n == nw - 1:
                x_copy(1).wait()
                for i in range(2, NX):
                    x_copy(i).start()
                pending += ln_first_tasks(SUB)
            per = WCHUNKS[n][1] // CW
            for t in pending:
                t()
            pending = []
            for k, (mm, post) in enumerate(pairs[pos:pos + per]):
                mm()
                if k + 1 < per or n == nw - 1:
                    post()
                else:
                    pending.append(post)
            pos += per
        kv_task()

    def p0_body(i, c):
        inext = jnp.minimum(i + 1, NX - 1)

        @pl.when(i + 1 < NX)
        def _():
            x_copy(inext).wait()

        @pl.when(i == 2)
        def _():
            cp_awo.start()
            cp_bwqkv.start()
            cp_bwo.start()
        r0 = _mult(i * SUB, SUB)
        h = lhs_pq(r0, SUB)
        tasks = qkv_a_tasks(lambda: h, 0, i)
        _interleave(tasks[:-1], ln_first_tasks(_mult(inext * SUB, SUB)))
        tasks[-1]()
        return c
    with _scope("P0"):
        lax.fori_loop(1, NX, p0_body, 0)
    cp_awo.wait()
    cp_bwqkv.wait()
    cp_bwo.wait()
    finish_kv()
    with _scope("P1"):
        proj_phase(lhs_pq, kvw_s, qkv_b_tasks, True, xio)
    with _scope("MHA"):
        attention(1, True, fin_extra(False, 1))

    def p2_step(i, nxt):
        ra, rb = rows_of(i)

        def out_next(u, dst):
            if nxt:
                r0 = rows_of(i + 1)[u]
                mm, get_h = out_tasks(lhs_o, bwo_p, r0, x_s)
                _interleave(mm, [])
                dst[_half(r0, SUB), :] = _pack(get_h())

        out_next(1, hb_s)
        _interleave(qkv_a_tasks(lambda: lhs_pq(ra, SUB), i, 0), [])
        out_next(0, pq_s)
        _interleave(qkv_a_tasks(lambda: _unpack(hb_s[_half(rb, SUB), :]), i, 1), [])

    def p2_body(i, c):
        p2_step(i, True)
        return c

    with _scope("P2"):
        lax.fori_loop(0, NT - 1, p2_body, 0)
        p2_step(NT - 1, False)
    finish_kv()
    with _scope("P1"):
        proj_phase(lhs_pq, kvw_s, qkv_b_tasks, True, x_s)

    with _scope("MHA"):
        attention(LAG, False, fin_extra(True, LAG))

    def out_copy(i):
        t0 = _mult(i * SUB, SUB)
        return pltpu.make_async_copy(xio.at[pl.ds(t0, SUB)], out_hbm.at[pl.ds(t0, SUB)], osems.at[i])

    def final_body(i, c):
        for u, r0 in enumerate(rows_of(i)):
            y = x_s[pl.ds(r0, SUB), :] + _dot(lhs_o(r0, SUB), _unpack(bwo_p[...]))
            xio[pl.ds(r0, SUB), :] = y.astype(BF16)
            out_copy(i * NSUB + u).start()
        return c
    for u in range(NSUB):
        out_copy(u).start()
    with _scope("P4"):
        lax.fori_loop(1, NT, final_body, 0)

    with _scope("waitout"):
        for i in range(NX):
            out_copy(i).wait()


@jax.jit
def pallas_interleave_layers__linear_attn_block__mha_block__prompt_kernel(
    A_x: jax.Array,
    A_wqkv: jax.Array,
    A_wo: jax.Array,
    B_x: jax.Array,
    B_wqkv: jax.Array,
    B_wo: jax.Array,
):
    del B_x
    x = A_x.reshape(S, D)
    any_spec = pl.BlockSpec(memory_space=pl.ANY)
    out = pl.pallas_call(
        _kernel,
        out_shape=jax.ShapeDtypeStruct((S, D), BF16),
        in_specs=[any_spec] * 5,
        out_specs=any_spec,
        scratch_shapes=[
            pltpu.VMEM((S, D), BF16),
            pltpu.VMEM((D, 3 * D), BF16),
            pltpu.VMEM((D, D), BF16),
            pltpu.VMEM((D, 3 * D), BF16),
            pltpu.VMEM((D, D), BF16),
            pltpu.VMEM((S, D), F32),
            pltpu.VMEM((S // 2, D), jnp.uint32),
            pltpu.VMEM((NG, S, 128), BF16),
            pltpu.VMEM((NT, D, TS), BF16),
            pltpu.VMEM((NT, D, TS), BF16),
            pltpu.VMEM((NG, S // 2, 128), jnp.uint32),
            pltpu.VMEM((LAG, 128, TQ), F32),
            pltpu.VMEM((NG, 128, 128), F32),
            pltpu.VMEM((8, D), F32),
            pltpu.VMEM((D, 128), F32),
            pltpu.VMEM((D // 2, D), jnp.uint32),
            pltpu.VMEM((NX, D, SUB), BF16),
            pltpu.VMEM((D // 2, D), jnp.uint32),
            pltpu.VMEM((S // 2, D), jnp.uint32),
            pltpu.VMEM((4 * LAG, 8, TQ), F32),
            pltpu.SemaphoreType.DMA((3,)),
            pltpu.SemaphoreType.DMA((len(WCHUNKS),)),
            pltpu.SemaphoreType.DMA((NX,)),
            pltpu.SemaphoreType.DMA((NX,)),
        ] + [pltpu.VMEM((S, TQ), F32)] * (4 * LAG),
        compiler_params=pltpu.CompilerParams(vmem_limit_bytes=120 * 1024 * 1024),
        name="interleave_layers",
    )(x, A_wqkv, A_wo, B_wqkv, B_wo)
    return out.reshape(1, S, D)
```

```python
import math

import jax
import jax.numpy as jnp
from jax import lax
import jax.experimental.pallas as pl
import jax.experimental.pallas.tpu as pltpu

S, D, H, DH = 2048, 1024, 32, 32
NG = D // 128
TS = 512
SUB = 256
NSUB = TS // SUB
NT = S // TS
NX = S // SUB
CW = 256
NCW = D // CW
LNR = 32
TQ = 512
TK = 128
NQ = S // TQ
NC = S // TK
NIT = NG * NQ
LAG = 2
WCHUNKS = ((1024, 256), (1280, 256), (1536, 512), (0, 512), (512, 512), (2048, 1024))
OSPLIT = ((0, 512), (512, 256), (768, 256))
QSCALE = (DH ** -0.5) * math.log2(math.e)
F32 = jnp.float32
BF16 = jnp.bfloat16
U32 = jnp.uint32


def _dot(a, b):
    return jnp.dot(a, b, preferred_element_type=F32)


def _ln_finish(x, s1, s2):
    mu = jnp.sum(s1, axis=-1, keepdims=True) * (1.0 / D)
    ms = jnp.sum(s2, axis=-1, keepdims=True) * (1.0 / D)
    var = jnp.maximum(ms - mu * mu, 0.0)
    return ((x - mu) * lax.rsqrt(var + 1e-5)).astype(BF16)


def _layernorm(x):
    return _ln_finish(x, x, x * x)


def _phi(t):
    return jnp.where(t > 0, t + 1.0, jnp.exp(t)) + 1e-6


def _recip(d):
    r = pl.reciprocal(d, approx=True)
    return r * (2.0 - d * r)


def _mult(v, m):
    return v if isinstance(v, int) else pl.multiple_of(v, m)


def _pack(v):
    return pltpu.bitcast(v, U32)


def _unpack(v):
    return pltpu.bitcast(v, BF16)


def _half(r0, n):
    return pl.ds(_mult(r0 // 2, n // 2), n // 2)


def _run(tasks):
    for t in tasks:
        t()


def _interleave(main, side):
    done = 0
    for n, task in enumerate(main):
        task()
        want = ((n + 1) * len(side)) // len(main)
        while done < want:
            side[done]()
            done += 1


def _rows_of(i):
    t0 = _mult(i * TS, TS)
    return [_mult(t0 + u * SUB, SUB) for u in range(NSUB)]


def _kernel(x_hbm, awqkv_hbm, awo_hbm, bwqkv_hbm, bwo_hbm, out_hbm,
            xio, awqkv, awo, bwqkv, bwo,
            x_s, pq_s, k_s, qt_s, vt_s, o_s, ott,
            g_s, z_s, zc_s, kvw_s, pqt_s, bwo_p, hb_s,
            m_s, sems, wsems, xsems, osem, *sb):

    def x_copy(i):
        t0 = _mult(i * SUB, SUB)
        return pltpu.make_async_copy(x_hbm.at[pl.ds(t0, SUB)], xio.at[pl.ds(t0, SUB)], xsems.at[i])

    def w_copy(n):
        c0, w = WCHUNKS[n]
        return pltpu.make_async_copy(awqkv_hbm.at[:, pl.ds(c0, w)],
                                     awqkv.at[:, pl.ds(c0, w)], wsems.at[n])

    cp_awo = pltpu.make_async_copy(awo_hbm, awo, sems.at[0])
    cp_bwqkv = pltpu.make_async_copy(bwqkv_hbm, bwqkv, sems.at[1])
    cp_bwo = pltpu.make_async_copy(bwo_hbm, bwo, sems.at[2])
    x_copy(0).start()
    w_copy(0).start()

    def qkv_a_tasks(get_h, ix, first=False):
        st = {}

        def mm(key, c0):
            def f():
                st[key] = _dot(get_h(), awqkv[:, c0:c0 + CW])
            return f

        def k_post(n):
            def f():
                c0 = n * CW
                pk = _phi(st["k", n])
                z_s[:, c0:c0 + CW] += jnp.sum(pk.reshape(SUB // 8, 8, CW), axis=0)
                st["k", n] = pk.T.astype(BF16)
            return f

        def q_post(n):
            def f():
                c0 = n * CW
                pqt_s[ix, c0:c0 + CW, :] = _phi(st["q", n]).T.astype(BF16)
            return f

        def g_task(n):
            def f():
                c0 = n * CW
                if first:
                    g_s[c0:c0 + CW, :] = _dot(st["k", n], get_h())
                else:
                    pkt = jnp.concatenate([st["k", m] for m in range(NCW)], axis=0)
                    g_s[:, c0:c0 + CW] += _dot(pkt, get_h()[:, c0:c0 + CW])
            return f

        pairs = ([(mm(("k", n), D + n * CW), k_post(n)) for n in range(NCW)]
                 + [(mm(("q", n), n * CW), q_post(n)) for n in range(NCW)])
        g_tasks = [g_task(n) for n in range(NCW)]
        if first:
            return pairs, g_tasks
        return [(lambda p=p: _run(p)) for p in pairs] + g_tasks

    def qkv_b_tasks(get_h, i, u):
        r0 = _rows_of(i)[u]
        cols = slice(u * SUB, (u + 1) * SUB)

        def v_task(n):
            def f():
                c0 = n * CW
                v = _dot(get_h(), bwqkv[:, 2 * D + c0:2 * D + c0 + CW])
                vt_s[i, c0:c0 + CW, cols] = v.T.astype(BF16)
            return f

        def q_task(n):
            def f():
                c0 = n * CW
                q = _dot(get_h(), bwqkv[:, c0:c0 + CW]) * QSCALE
                qt_s[i, c0:c0 + CW, cols] = q.T.astype(BF16)
            return f

        def k_task(n):
            def f():
                c0 = n * CW
                k = _dot(get_h(), bwqkv[:, D + c0:D + c0 + CW]).astype(BF16)
                for t in range(CW // 128):
                    k_s[c0 // 128 + t, pl.ds(r0, SUB), :] = k[:, t * 128:(t + 1) * 128]
            return f

        order = (k_task, v_task, q_task) if u == 0 else (v_task, q_task, k_task)
        return [t(n) for t in order for n in range(NCW)]

    def out_ln(lhs, w_ref, r0, res_ref):
        s1 = s2 = None
        for n in range(NCW):
            c0 = n * CW
            x = res_ref[pl.ds(r0, SUB), c0:c0 + CW].astype(F32) + _dot(
                lhs(r0, SUB), _unpack(w_ref[:, c0:c0 + CW]))
            x_s[pl.ds(r0, SUB), c0:c0 + CW] = x
            for u in range(CW // 128):
                xu = x[:, u * 128:(u + 1) * 128]
                s1 = xu if s1 is None else s1 + xu
                s2 = xu * xu if s2 is None else s2 + xu * xu
        return _ln_finish(x_s[pl.ds(r0, SUB), :], s1, s2)

    def lhs_pq(r0, n):
        return _unpack(pq_s[_half(r0, n), :])

    def lhs_o(r0, n, g0=0, g1=NG):
        return _unpack(jnp.concatenate([o_s[g, _half(r0, n), :] for g in range(g0, g1)], axis=1))

    def norm_pq_tasks(i):
        def task(u, n):
            def f():
                c0 = _mult(i * TS + u * 128, 128)
                ix, lo = divmod(u * 128, SUB)
                nh = CW // DH
                rows = slice(n * CW, (n + 1) * CW)
                pqt = pqt_s[i * NSUB + ix, rows, lo:lo + 128].astype(F32).reshape(nh, DH, 128)
                den = jnp.sum(pqt * zc_s[rows, :].reshape(nh, DH, 128), axis=1, keepdims=True) + 1e-6
                pn = (pqt * _recip(den)).reshape(CW, 128)
                pq_s[_half(c0, 128), rows] = _pack(pn.T.astype(BF16))
            return f
        return [task(u, n) for u in range(TS // 128) for n in range(NCW)]

    def finish_kv():
        ri = lax.broadcasted_iota(jnp.int32, (128, 128), 0) // DH
        ci = lax.broadcasted_iota(jnp.int32, (128, 128), 1) // DH
        diag = ri == ci
        z = jnp.sum(z_s[...], axis=0, keepdims=True)
        zc_s[...] = jnp.broadcast_to(z, (128, D)).T

        kvs = [_dot(g_s[g * 128:(g + 1) * 128, :].astype(BF16),
                    awqkv[:, 2 * D + g * 128:2 * D + (g + 1) * 128]) for g in range(NG)]

        def kvw(g):
            def f():
                kvd = jnp.where(diag, kvs[g], 0.0).astype(BF16)
                kvw_s[g * 64:(g + 1) * 64, :] = _pack(
                    _dot(kvd, awo[g * 128:(g + 1) * 128, :]).astype(BF16))
            return f
        _interleave([kvw(g) for g in range(NG)], norm_pq_tasks(0))

    def ln_tasks(r0, src=xio, rows=SUB, dst=pq_s):
        def task(p):
            def f():
                rr = _mult(r0 + p * LNR, LNR)
                x = src[pl.ds(rr, LNR), :].astype(F32)
                dst[_half(rr, LNR), :] = _pack(_layernorm(x))
            return f
        return [task(p) for p in range(rows // LNR)]

    def lin_out_mha_in(first):
        res_ref = xio if first else x_s

        def body(i, c):
            ra, rb = _rows_of(i)
            h_a = out_ln(lhs_pq, kvw_s, ra, res_ref)
            h_b = out_ln(lhs_pq, kvw_s, rb, res_ref)
            _run(norm_pq_tasks(jnp.minimum(i + 1, NT - 1)))
            _run(qkv_b_tasks(lambda: h_a, i, 0))
            if first:
                w0 = _mult(i * (D // NT), D // NT)
                bwo_p[_half(w0, D // NT), :] = _pack(bwo[pl.ds(w0, D // NT), :])
                g_s[pl.ds(w0, D // NT), :] = jnp.zeros((D // NT, D), F32)
            _run(qkv_b_tasks(lambda: h_b, i, 1))
            return c
        lax.fori_loop(0, NT, body, 0)

    def make_w(g, j, qi):
        r0 = _mult(g * 128 + j * DH, DH)
        parts = []
        if j > 0:
            parts.append(jnp.zeros((DH * j, TQ), BF16))
        parts.append(qt_s[qi, pl.ds(r0, DH), :])
        if j < 3:
            parts.append(jnp.zeros((DH * (3 - j), TQ), BF16))
        return jnp.concatenate(parts, axis=0)

    def s1_store(c, s, sbuf, m8):
        sbuf[c * TK:(c + 1) * TK, :] = s
        for r in range(TK // 8):
            blk = s[r * 8:(r + 1) * 8, :]
            m8 = blk if m8 is None else jnp.maximum(m8, blk)
        return m8

    def s2_chunk(c, m, r0, sbuf, l8, acc):
        p = jnp.exp2(sbuf[c * TK:(c + 1) * TK, :] - m)
        for r in reversed(range(TK // 16)):
            ab = p[r * 16:r * 16 + 8, :] + p[r * 16 + 8:r * 16 + 16, :]
            l8 = ab if l8 is None else l8 + ab
        ti, lo = divmod(c * TK, TS)
        o = _dot(vt_s[ti, pl.ds(r0, DH), lo:lo + TK], p.astype(BF16))
        return l8, (o if acc is None else o + acc)

    def item(it):
        return it % NG, it // NG

    def flush_o(prev, slot):
        g, qi = prev
        o_s[g, _half(qi * TQ, TQ), :] = _pack(ott[slot].T.astype(BF16))

    def attn_step(prev, cur, nxt, slot, extra=()):
        extra = list(extra)
        every = (4 * NC) // len(extra) if extra else 0
        if prev is not None:
            flush_o(prev, slot)
        for j in range(4):
            b = slot * 4 + j
            if cur is not None:
                r0 = _mult(cur[0] * 128 + j * DH, DH)
                m = m_s[b, 0:1, :]
            if nxt is not None:
                w = make_w(nxt[0], j, nxt[1])
            m8 = l8 = acc = None
            for c in range(NC):
                if extra and (j * NC + c) % every == 0:
                    extra.pop(0)()
                if nxt is not None:
                    s = _dot(k_s[nxt[0], c * TK:(c + 1) * TK, :], w)
                if cur is not None:
                    l8, acc = s2_chunk(c, m, r0, sb[b], l8, acc)
                if nxt is not None:
                    m8 = s1_store(c, s, sb[b], m8)
            if cur is not None:
                l = jnp.sum(l8, axis=0, keepdims=True)
                ott[slot, j * DH:(j + 1) * DH, :] = acc * _recip(l)
            if nxt is not None:
                m_s[b] = jnp.broadcast_to(jnp.max(m8, axis=0, keepdims=True), (8, TQ))

    def tail_pieces(last, lag):
        pr = 128 // lag

        def pieces(r0, c0):
            st = {}

            def f0():
                st["p"] = (_dot(lhs_o(r0, pr, 0, 4), _unpack(bwo_p[0:256, c0:c0 + 128]))
                           + x_s[r0:r0 + pr, c0:c0 + 128])

            def f1():
                y = _dot(lhs_o(r0, pr, 4, 8), _unpack(bwo_p[256:512, c0:c0 + 128])) + st["p"]
                if last:
                    xio[r0:r0 + pr, c0:c0 + 128] = y.astype(BF16)
                else:
                    x_s[r0:r0 + pr, c0:c0 + 128] = y
                    if c0 + 128 == D:
                        _run(ln_tasks(r0, x_s, pr, (pq_s, hb_s)[(r0 // SUB) % 2]))
            return [f0, f1]
        return [f for r0 in range(0, TS, pr) for c0 in range(0, D, 128) for f in pieces(r0, c0)]

    def attention(lag, last):
        for u in range(lag):
            attn_step(None, None, item(u), u)
        ott[...] = jnp.zeros(ott.shape, F32)
        if not last:
            z_s[...] = jnp.zeros(z_s.shape, F32)

        def body(ib, c):
            for u in range(lag):
                it = ib * lag + u
                attn_step(item(jnp.maximum(ib - 1, 0) * lag + u), item(it), item(it + lag), u)
            return c
        lax.fori_loop(0, NIT // lag - 1, body, 0)
        extra = tail_pieces(last, lag)
        ne = len(extra) // lag
        for u in range(lag):
            it = NIT - lag + u
            attn_step(item(it - lag), item(it), None, u, extra[u * ne:(u + 1) * ne])
        for u in range(lag):
            flush_o(item(NIT - lag + u), u)

    z_s[...] = jnp.zeros(z_s.shape, F32)
    x_copy(0).wait()
    w_copy(1).start()
    _run(ln_tasks(0))
    h0 = lhs_pq(0, SUB)
    pairs, g_tasks = qkv_a_tasks(lambda: h0, 0, first=True)
    w_copy(0).wait()
    w_copy(2).start()
    pairs[0][0]()
    w_copy(1).wait()
    w_copy(3).start()
    pairs[0][1]()
    pairs[1][0]()
    g_tasks[0]()
    w_copy(2).wait()
    x_copy(1).start()
    w_copy(4).start()
    pairs[1][1]()
    _run(pairs[2] + pairs[3])
    g_tasks[1]()
    w_copy(3).wait()
    _run(pairs[4] + pairs[5])
    g_tasks[2]()
    w_copy(4).wait()
    x_copy(1).wait()
    for i in range(2, NX):
        x_copy(i).start()
    _run(ln_tasks(SUB))
    _run(pairs[6] + pairs[7])
    g_tasks[3]()

    def p0_body(i, c):
        inext = jnp.minimum(i + 1, NX - 1)

        @pl.when(i + 1 < NX)
        def _():
            x_copy(inext).wait()

        @pl.when(i == 2)
        def _():
            w_copy(5).start()
            cp_awo.start()
            cp_bwqkv.start()
            cp_bwo.start()
        h = lhs_pq(_mult(i * SUB, SUB), SUB)
        _interleave(qkv_a_tasks(lambda: h, i), ln_tasks(_mult(inext * SUB, SUB)))
        return c
    lax.fori_loop(1, NX, p0_body, 0)
    w_copy(5).wait()
    cp_awo.wait()
    cp_bwqkv.wait()
    cp_bwo.wait()
    finish_kv()

    lin_out_mha_in(True)
    attention(1, False)

    def p2_step(i, nxt):
        ra, rb = _rows_of(i)

        def out_next(u, dst):
            if nxt:
                r0 = _rows_of(i + 1)[u]
                dst[_half(r0, SUB), :] = _pack(out_ln(lhs_o, bwo_p, r0, x_s))

        out_next(1, hb_s)
        _run(qkv_a_tasks(lambda: lhs_pq(ra, SUB), i * NSUB))
        out_next(0, pq_s)
        _run(qkv_a_tasks(lambda: _unpack(hb_s[_half(rb, SUB), :]), i * NSUB + 1))

    def p2_body(i, c):
        p2_step(i, True)
        return c
    lax.fori_loop(0, NT - 1, p2_body, 0)
    p2_step(NT - 1, False)
    finish_kv()

    lin_out_mha_in(False)
    attention(LAG, True)

    def out_copy(r0, n, c0=0, w=D):
        return pltpu.make_async_copy(xio.at[pl.ds(r0, n), pl.ds(c0, w)],
                                     out_hbm.at[pl.ds(r0, n), pl.ds(c0, w)], osem)

    def final_body(i, c):
        ra, rb = _rows_of(i)
        y = x_s[pl.ds(ra, SUB), :] + _dot(lhs_o(ra, SUB), _unpack(bwo_p[...]))
        xio[pl.ds(ra, SUB), :] = y.astype(BF16)
        out_copy(ra, SUB).start()
        for c0, w in OSPLIT:
            y = x_s[pl.ds(rb, SUB), c0:c0 + w] + _dot(lhs_o(rb, SUB), _unpack(bwo_p[:, c0:c0 + w]))
            xio[pl.ds(rb, SUB), c0:c0 + w] = y.astype(BF16)
            out_copy(rb, SUB, c0, w).start()
        return c
    out_copy(0, TS).start()
    lax.fori_loop(1, NT, final_body, 0)
    out_copy(0, S).wait()


@jax.jit
def pallas_interleave_layers__linear_attn_block__mha_block__prompt_kernel(
    A_x: jax.Array,
    A_wqkv: jax.Array,
    A_wo: jax.Array,
    B_x: jax.Array,
    B_wqkv: jax.Array,
    B_wo: jax.Array,
):
    del B_x
    x = A_x.reshape(S, D)
    any_spec = pl.BlockSpec(memory_space=pl.ANY)
    out = pl.pallas_call(
        _kernel,
        out_shape=jax.ShapeDtypeStruct((S, D), BF16),
        in_specs=[any_spec] * 5,
        out_specs=any_spec,
        scratch_shapes=[
            pltpu.VMEM((S, D), BF16),
            pltpu.VMEM((D, 3 * D), BF16),
            pltpu.VMEM((D, D), BF16),
            pltpu.VMEM((D, 3 * D), BF16),
            pltpu.VMEM((D, D), BF16),
            pltpu.VMEM((S, D), F32),
            pltpu.VMEM((S // 2, D), U32),
            pltpu.VMEM((NG, S, 128), BF16),
            pltpu.VMEM((NT, D, TS), BF16),
            pltpu.VMEM((NT, D, TS), BF16),
            pltpu.VMEM((NG, S // 2, 128), U32),
            pltpu.VMEM((LAG, 128, TQ), F32),
            pltpu.VMEM((D, D), F32),
            pltpu.VMEM((8, D), F32),
            pltpu.VMEM((D, 128), F32),
            pltpu.VMEM((D // 2, D), U32),
            pltpu.VMEM((NX, D, SUB), BF16),
            pltpu.VMEM((D // 2, D), U32),
            pltpu.VMEM((S // 2, D), U32),
            pltpu.VMEM((4 * LAG, 8, TQ), F32),
            pltpu.SemaphoreType.DMA((3,)),
            pltpu.SemaphoreType.DMA((len(WCHUNKS),)),
            pltpu.SemaphoreType.DMA((NX,)),
            pltpu.SemaphoreType.DMA(()),
        ] + [pltpu.VMEM((S, TQ), F32)] * (4 * LAG),
        compiler_params=pltpu.CompilerParams(vmem_limit_bytes=120 * 1024 * 1024),
        name="interleave_layers",
    )(x, A_wqkv, A_wo, B_wqkv, B_wo)
    return out.reshape(1, S, D)
```

```python
import math

import jax
import jax.numpy as jnp
from jax import lax
import jax.experimental.pallas as pl
import jax.experimental.pallas.tpu as pltpu

S, D, H, DH = 2048, 1024, 32, 32
NG = D // 128
TS = 512
SUB = 256
NSUB = TS // SUB
NT = S // TS
NX = S // SUB
CW = 256
NCW = D // CW
LNR = 32
TQ = 512
TK = 128
NQ = S // TQ
NC = S // TK
NIT = NG * NQ
LAG = 2
WCHUNKS = ((1024, 256), (1280, 256), (1536, 512), (0, 512), (512, 512), (2048, 1024))
OSPLIT = ((0, 512), (512, 256), (768, 256))
QSCALE = (DH ** -0.5) * math.log2(math.e)
F32 = jnp.float32
BF16 = jnp.bfloat16
U32 = jnp.uint32


def _dot(a, b):
    return jnp.dot(a, b, preferred_element_type=F32)


def _ln_finish(x, s1, s2):
    mu = jnp.sum(s1, axis=-1, keepdims=True) * (1.0 / D)
    ms = jnp.sum(s2, axis=-1, keepdims=True) * (1.0 / D)
    var = jnp.maximum(ms - mu * mu, 0.0)
    return ((x - mu) * lax.rsqrt(var + 1e-5)).astype(BF16)


def _layernorm(x):
    return _ln_finish(x, x, x * x)


def _phi(t):
    return jnp.where(t > 0, t + 1.0, jnp.exp(t)) + 1e-6


def _recip(d):
    r = pl.reciprocal(d, approx=True)
    return r * (2.0 - d * r)


def _mult(v, m):
    return v if isinstance(v, int) else pl.multiple_of(v, m)


def _pack(v):
    return pltpu.bitcast(v, U32)


def _unpack(v):
    return pltpu.bitcast(v, BF16)


def _half(r0, n):
    return pl.ds(_mult(r0 // 2, n // 2), n // 2)


def _run(tasks):
    for t in tasks:
        t()


def _interleave(main, side):
    done = 0
    for n, task in enumerate(main):
        task()
        want = ((n + 1) * len(side)) // len(main)
        while done < want:
            side[done]()
            done += 1


def _rows_of(i):
    t0 = _mult(i * TS, TS)
    return [_mult(t0 + u * SUB, SUB) for u in range(NSUB)]


def _kernel(x_hbm, awqkv_hbm, awo_hbm, bwqkv_hbm, bwo_hbm, out_hbm,
            xio, awqkv, awo, bwqkv, bwo,
            x_s, pq_s, k_s, qt_s, vt_s, o_s, ott,
            g_s, z_s, zc_s, kvw_s, pqt_s, bwo_p,
            m_s, sems, wsems, xsems, osem, *sb):

    def x_copy(i):
        t0 = _mult(i * SUB, SUB)
        return pltpu.make_async_copy(x_hbm.at[pl.ds(t0, SUB)], xio.at[pl.ds(t0, SUB)], xsems.at[i])

    def w_copy(n):
        c0, w = WCHUNKS[n]
        return pltpu.make_async_copy(awqkv_hbm.at[:, pl.ds(c0, w)],
                                     awqkv.at[:, pl.ds(c0, w)], wsems.at[n])

    cp_awo = pltpu.make_async_copy(awo_hbm, awo, sems.at[0])
    cp_bwqkv = pltpu.make_async_copy(bwqkv_hbm, bwqkv, sems.at[1])
    cp_bwo = pltpu.make_async_copy(bwo_hbm, bwo, sems.at[2])
    x_copy(0).start()
    w_copy(0).start()

    def qkv_a_tasks(get_h, ix, first=False):
        st = {}

        def mm(key, c0):
            def f():
                st[key] = _dot(get_h(), awqkv[:, c0:c0 + CW])
            return f

        def k_post(n):
            def f():
                c0 = n * CW
                pk = _phi(st["k", n])
                z_s[:, c0:c0 + CW] += jnp.sum(pk.reshape(SUB // 8, 8, CW), axis=0)
                st["k", n] = pk.T.astype(BF16)
            return f

        def q_post(n):
            def f():
                c0 = n * CW
                pqt_s[ix, c0:c0 + CW, :] = _phi(st["q", n]).T.astype(BF16)
            return f

        def g_task(n):
            def f():
                c0 = n * CW
                if first:
                    g_s[c0:c0 + CW, :] = _dot(st["k", n], get_h())
                else:
                    pkt = jnp.concatenate([st["k", m] for m in range(NCW)], axis=0)
                    g_s[:, c0:c0 + CW] += _dot(pkt, get_h()[:, c0:c0 + CW])
            return f

        pairs = ([(mm(("k", n), D + n * CW), k_post(n)) for n in range(NCW)]
                 + [(mm(("q", n), n * CW), q_post(n)) for n in range(NCW)])
        g_tasks = [g_task(n) for n in range(NCW)]
        if first:
            return pairs, g_tasks
        return [(lambda p=p: _run(p)) for p in pairs] + g_tasks

    def qkv_b_tasks(get_h, i, u):
        r0 = _rows_of(i)[u]
        cols = slice(u * SUB, (u + 1) * SUB)

        def v_task(n):
            def f():
                c0 = n * CW
                v = _dot(get_h(), bwqkv[:, 2 * D + c0:2 * D + c0 + CW])
                vt_s[i, c0:c0 + CW, cols] = v.T.astype(BF16)
            return f

        def q_task(n):
            def f():
                c0 = n * CW
                q = _dot(get_h(), bwqkv[:, c0:c0 + CW]) * QSCALE
                qt_s[i, c0:c0 + CW, cols] = q.T.astype(BF16)
            return f

        def k_task(n):
            def f():
                c0 = n * CW
                k = _dot(get_h(), bwqkv[:, D + c0:D + c0 + CW]).astype(BF16)
                for t in range(CW // 128):
                    k_s[c0 // 128 + t, pl.ds(r0, SUB), :] = k[:, t * 128:(t + 1) * 128]
            return f

        order = (k_task, v_task, q_task) if u == 0 else (v_task, q_task, k_task)
        return [t(n) for t in order for n in range(NCW)]

    def out_ln(lhs, w_ref, r0, res_ref):
        s1 = s2 = None
        for n in range(NCW):
            c0 = n * CW
            x = res_ref[pl.ds(r0, SUB), c0:c0 + CW].astype(F32) + _dot(
                lhs(r0, SUB), _unpack(w_ref[:, c0:c0 + CW]))
            x_s[pl.ds(r0, SUB), c0:c0 + CW] = x
            for u in range(CW // 128):
                xu = x[:, u * 128:(u + 1) * 128]
                s1 = xu if s1 is None else s1 + xu
                s2 = xu * xu if s2 is None else s2 + xu * xu
        return _ln_finish(x_s[pl.ds(r0, SUB), :], s1, s2)

    def lhs_pq(r0, n):
        return _unpack(pq_s[_half(r0, n), :])

    def lhs_o(r0, n, g0=0, g1=NG):
        return _unpack(jnp.concatenate([o_s[g, _half(r0, n), :] for g in range(g0, g1)], axis=1))

    def norm_pq_tasks(i):
        def task(u, n):
            def f():
                c0 = _mult(i * TS + u * 128, 128)
                ix, lo = divmod(u * 128, SUB)
                nh = CW // DH
                rows = slice(n * CW, (n + 1) * CW)
                pqt = pqt_s[i * NSUB + ix, rows, lo:lo + 128].astype(F32).reshape(nh, DH, 128)
                den = jnp.sum(pqt * zc_s[rows, :].reshape(nh, DH, 128), axis=1, keepdims=True) + 1e-6
                pn = (pqt * _recip(den)).reshape(CW, 128)
                pq_s[_half(c0, 128), rows] = _pack(pn.T.astype(BF16))
            return f
        return [task(u, n) for u in range(TS // 128) for n in range(NCW)]

    def finish_kv():
        ri = lax.broadcasted_iota(jnp.int32, (128, 128), 0) // DH
        ci = lax.broadcasted_iota(jnp.int32, (128, 128), 1) // DH
        diag = ri == ci
        z = jnp.sum(z_s[...], axis=0, keepdims=True)
        zc_s[...] = jnp.broadcast_to(z, (128, D)).T

        kvs = [_dot(g_s[g * 128:(g + 1) * 128, :].astype(BF16),
                    awqkv[:, 2 * D + g * 128:2 * D + (g + 1) * 128]) for g in range(NG)]

        def kvw(g):
            def f():
                kvd = jnp.where(diag, kvs[g], 0.0).astype(BF16)
                kvw_s[g * 64:(g + 1) * 64, :] = _pack(
                    _dot(kvd, awo[g * 128:(g + 1) * 128, :]).astype(BF16))
            return f
        _interleave([kvw(g) for g in range(NG)], norm_pq_tasks(0))

    def ln_tasks(r0, src=xio, rows=SUB):
        def task(p):
            def f():
                rr = _mult(r0 + p * LNR, LNR)
                x = src[pl.ds(rr, LNR), :].astype(F32)
                pq_s[_half(rr, LNR), :] = _pack(_layernorm(x))
            return f
        return [task(p) for p in range(rows // LNR)]

    def lin_out_mha_in(first):
        res_ref = xio if first else x_s

        def body(i, c):
            ra, rb = _rows_of(i)
            h_a = out_ln(lhs_pq, kvw_s, ra, res_ref)
            h_b = out_ln(lhs_pq, kvw_s, rb, res_ref)
            _run(norm_pq_tasks(jnp.minimum(i + 1, NT - 1)))
            _run(qkv_b_tasks(lambda: h_a, i, 0))
            if first:
                w0 = _mult(i * (D // NT), D // NT)
                bwo_p[_half(w0, D // NT), :] = _pack(bwo[pl.ds(w0, D // NT), :])
                g_s[pl.ds(w0, D // NT), :] = jnp.zeros((D // NT, D), F32)
            _run(qkv_b_tasks(lambda: h_b, i, 1))
            return c
        lax.fori_loop(0, NT, body, 0)

    def make_w(g, j, qi):
        r0 = _mult(g * 128 + j * DH, DH)
        parts = []
        if j > 0:
            parts.append(jnp.zeros((DH * j, TQ), BF16))
        parts.append(qt_s[qi, pl.ds(r0, DH), :])
        if j < 3:
            parts.append(jnp.zeros((DH * (3 - j), TQ), BF16))
        return jnp.concatenate(parts, axis=0)

    def s1_store(c, s, sbuf, m8):
        sbuf[c * TK:(c + 1) * TK, :] = s
        for r in range(TK // 8):
            blk = s[r * 8:(r + 1) * 8, :]
            m8 = blk if m8 is None else jnp.maximum(m8, blk)
        return m8

    def s2_chunk(c, m, r0, sbuf, l8, acc):
        p = jnp.exp2(sbuf[c * TK:(c + 1) * TK, :] - m)
        for r in reversed(range(TK // 16)):
            ab = p[r * 16:r * 16 + 8, :] + p[r * 16 + 8:r * 16 + 16, :]
            l8 = ab if l8 is None else l8 + ab
        ti, lo = divmod(c * TK, TS)
        o = _dot(vt_s[ti, pl.ds(r0, DH), lo:lo + TK], p.astype(BF16))
        return l8, (o if acc is None else o + acc)

    def item(it):
        return it % NG, it // NG

    def flush_o(prev, slot):
        g, qi = prev
        o_s[g, _half(qi * TQ, TQ), :] = _pack(ott[slot].T.astype(BF16))

    def attn_step(prev, cur, nxt, slot, extra=()):
        extra = list(extra)
        every = (4 * NC) // len(extra) if extra else 0
        if prev is not None:
            flush_o(prev, slot)
        for j in range(4):
            b = slot * 4 + j
            if cur is not None:
                r0 = _mult(cur[0] * 128 + j * DH, DH)
                m = m_s[b, 0:1, :]
            if nxt is not None:
                w = make_w(nxt[0], j, nxt[1])
            m8 = l8 = acc = None
            for c in range(NC):
                if extra and (j * NC + c) % every == 0:
                    extra.pop(0)()
                if nxt is not None:
                    s = _dot(k_s[nxt[0], c * TK:(c + 1) * TK, :], w)
                if cur is not None:
                    l8, acc = s2_chunk(c, m, r0, sb[b], l8, acc)
                if nxt is not None:
                    m8 = s1_store(c, s, sb[b], m8)
            if cur is not None:
                l = jnp.sum(l8, axis=0, keepdims=True)
                ott[slot, j * DH:(j + 1) * DH, :] = acc * _recip(l)
            if nxt is not None:
                m_s[b] = jnp.broadcast_to(jnp.max(m8, axis=0, keepdims=True), (8, TQ))

    def tail_pieces(last):
        pr = 128 // LAG

        def pieces(r0, c0):
            st = {}

            def f0():
                st["p"] = (_dot(lhs_o(r0, pr, 0, 4), _unpack(bwo_p[0:256, c0:c0 + 128]))
                           + x_s[r0:r0 + pr, c0:c0 + 128])

            def f1():
                y = _dot(lhs_o(r0, pr, 4, 8), _unpack(bwo_p[256:512, c0:c0 + 128])) + st["p"]
                if last:
                    xio[r0:r0 + pr, c0:c0 + 128] = y.astype(BF16)
                else:
                    x_s[r0:r0 + pr, c0:c0 + 128] = y
                    if c0 + 128 == D:
                        _run(ln_tasks(r0, x_s, pr))
            return [f0, f1]
        return [f for r0 in range(0, TS, pr) for c0 in range(0, D, 128) for f in pieces(r0, c0)]

    def attention(last):
        for u in range(LAG):
            attn_step(None, None, item(u), u)
        ott[...] = jnp.zeros(ott.shape, F32)
        if not last:
            z_s[...] = jnp.zeros(z_s.shape, F32)

        def body(ib, c):
            for u in range(LAG):
                it = ib * LAG + u
                attn_step(item(jnp.maximum(ib - 1, 0) * LAG + u), item(it), item(it + LAG), u)
            return c
        lax.fori_loop(0, NIT // LAG - 1, body, 0)
        extra = tail_pieces(last)
        ne = len(extra) // LAG
        for u in range(LAG):
            it = NIT - LAG + u
            attn_step(item(it - LAG), item(it), None, u, extra[u * ne:(u + 1) * ne])
        for u in range(LAG):
            flush_o(item(NIT - LAG + u), u)

    z_s[...] = jnp.zeros(z_s.shape, F32)
    x_copy(0).wait()
    w_copy(1).start()
    _run(ln_tasks(0))
    h0 = lhs_pq(0, SUB)
    pairs, g_tasks = qkv_a_tasks(lambda: h0, 0, first=True)
    w_copy(0).wait()
    w_copy(2).start()
    pairs[0][0]()
    w_copy(1).wait()
    w_copy(3).start()
    pairs[0][1]()
    pairs[1][0]()
    g_tasks[0]()
    w_copy(2).wait()
    x_copy(1).start()
    w_copy(4).start()
    pairs[1][1]()
    _run(pairs[2] + pairs[3])
    g_tasks[1]()
    w_copy(3).wait()
    _run(pairs[4] + pairs[5])
    g_tasks[2]()
    w_copy(4).wait()
    x_copy(1).wait()
    for i in range(2, NX):
        x_copy(i).start()
    _run(ln_tasks(SUB))
    _run(pairs[6] + pairs[7])
    g_tasks[3]()

    def p0_body(i, c):
        inext = jnp.minimum(i + 1, NX - 1)

        @pl.when(i + 1 < NX)
        def _():
            x_copy(inext).wait()

        @pl.when(i == 2)
        def _():
            w_copy(5).start()
            cp_awo.start()
            cp_bwqkv.start()
            cp_bwo.start()
        h = lhs_pq(_mult(i * SUB, SUB), SUB)
        _interleave(qkv_a_tasks(lambda: h, i), ln_tasks(_mult(inext * SUB, SUB)))
        return c
    lax.fori_loop(1, NX, p0_body, 0)
    w_copy(5).wait()
    cp_awo.wait()
    cp_bwqkv.wait()
    cp_bwo.wait()
    finish_kv()

    lin_out_mha_in(True)
    attention(False)

    def p2_body(ix, c):
        h = lhs_pq(_mult(ix * SUB, SUB), SUB)
        r0 = _mult((ix + NSUB) * SUB, SUB)
        tasks = qkv_a_tasks(lambda: h, ix)
        _run(tasks[:NCW])
        pq_s[_half(r0, SUB), :] = _pack(out_ln(lhs_o, bwo_p, r0, x_s))
        _run(tasks[NCW:])
        return c
    lax.fori_loop(0, NX - NSUB, p2_body, 0)
    for ix in range(NX - NSUB, NX):
        _run(qkv_a_tasks(lambda: lhs_pq(ix * SUB, SUB), ix))
    finish_kv()

    lin_out_mha_in(False)
    attention(True)

    def out_copy(r0, n, c0=0, w=D):
        return pltpu.make_async_copy(xio.at[pl.ds(r0, n), pl.ds(c0, w)],
                                     out_hbm.at[pl.ds(r0, n), pl.ds(c0, w)], osem)

    def final_body(i, c):
        ra, rb = _rows_of(i)
        y = x_s[pl.ds(ra, SUB), :] + _dot(lhs_o(ra, SUB), _unpack(bwo_p[...]))
        xio[pl.ds(ra, SUB), :] = y.astype(BF16)
        out_copy(ra, SUB).start()
        for c0, w in OSPLIT:
            y = x_s[pl.ds(rb, SUB), c0:c0 + w] + _dot(lhs_o(rb, SUB), _unpack(bwo_p[:, c0:c0 + w]))
            xio[pl.ds(rb, SUB), c0:c0 + w] = y.astype(BF16)
            out_copy(rb, SUB, c0, w).start()
        return c
    out_copy(0, TS).start()
    lax.fori_loop(1, NT, final_body, 0)
    out_copy(0, S).wait()


@jax.jit
def pallas_interleave_layers__linear_attn_block__mha_block__prompt_kernel(
    A_x: jax.Array,
    A_wqkv: jax.Array,
    A_wo: jax.Array,
    B_x: jax.Array,
    B_wqkv: jax.Array,
    B_wo: jax.Array,
):
    del B_x
    x = A_x.reshape(S, D)
    any_spec = pl.BlockSpec(memory_space=pl.ANY)
    out = pl.pallas_call(
        _kernel,
        out_shape=jax.ShapeDtypeStruct((S, D), BF16),
        in_specs=[any_spec] * 5,
        out_specs=any_spec,
        scratch_shapes=[
            pltpu.VMEM((S, D), BF16),
            pltpu.VMEM((D, 3 * D), BF16),
            pltpu.VMEM((D, D), BF16),
            pltpu.VMEM((D, 3 * D), BF16),
            pltpu.VMEM((D, D), BF16),
            pltpu.VMEM((S, D), F32),
            pltpu.VMEM((S // 2, D), U32),
            pltpu.VMEM((NG, S, 128), BF16),
            pltpu.VMEM((NT, D, TS), BF16),
            pltpu.VMEM((NT, D, TS), BF16),
            pltpu.VMEM((NG, S // 2, 128), U32),
            pltpu.VMEM((LAG, 128, TQ), F32),
            pltpu.VMEM((D, D), F32),
            pltpu.VMEM((8, D), F32),
            pltpu.VMEM((D, 128), F32),
            pltpu.VMEM((D // 2, D), U32),
            pltpu.VMEM((NX, D, SUB), BF16),
            pltpu.VMEM((D // 2, D), U32),
            pltpu.VMEM((4 * LAG, 8, TQ), F32),
            pltpu.SemaphoreType.DMA((3,)),
            pltpu.SemaphoreType.DMA((len(WCHUNKS),)),
            pltpu.SemaphoreType.DMA((NX,)),
            pltpu.SemaphoreType.DMA(()),
        ] + [pltpu.VMEM((S, TQ), F32)] * (4 * LAG),
        compiler_params=pltpu.CompilerParams(vmem_limit_bytes=120 * 1024 * 1024),
        name="interleave_layers",
    )(x, A_wqkv, A_wo, B_wqkv, B_wo)
    return out.reshape(1, S, D)
```
